```python
import jax
import jax.numpy as jnp

def _softmax(x, axis=-1):
    return jax.nn.softmax(x, axis=axis)
def _gelu(x):
    return jax.nn.gelu(x, approximate=True)
def _silu(x):
    return jax.nn.silu(x)
def _sigmoid(x):
    return jax.nn.sigmoid(x)
def _layernorm(x, axis=-1, eps=1e-5):
    m = jnp.mean(x, axis=axis, keepdims=True)
    v = jnp.var(x, axis=axis, keepdims=True)
    return (x - m) / jnp.sqrt(v + eps)
def _scatter_add(tgt, idx, src, axis=0):
    return tgt.at[idx].add(src)
def _segment_sum(src, seg, n):
    return jax.ops.segment_sum(src, seg, n)
class _Rng:
    def __init__(self, key):
        self._k = key
    def _next(self):
        self._k, sub = jax.random.split(self._k)
        return sub
    def normal(self, shape):
        return jax.random.normal(self._next(), shape, dtype=jnp.bfloat16)
    def randint(self, lo, hi, shape):
        return jax.random.randint(self._next(), shape, lo, hi, dtype=jnp.int32)
    def uniform(self, shape, lo=0.0, hi=1.0):
        return jax.random.uniform(self._next(), shape, jnp.bfloat16, lo, hi)
    def permutation(self, n):
        return jax.random.permutation(self._next(), n)


kernel_name = 'recurrent_scan__sliding_block_cached__moe_arch_mod__decode'

def setup_inputs():
    _rng = _Rng(jax.random.key(int.from_bytes(__import__("os").urandom(4), "little")))
    _w = (lambda a: (lambda t: t.astype(jnp.bfloat16) if jnp.issubdtype(t.dtype, jnp.floating) else t)(jnp.asarray(a)))
    def _A_setup():
        B, Sq, D = 1, 1, 512
        Hq, Hkv, Sk, Dh = 32, 32, 32768, 128
        assert Hq % Hkv == 0, (Hq, Hkv)
        return {
            "x": _w((lambda *s: _rng.normal(s) * 0.05)(B, Sq, D)),
            "k_cache": _w((lambda *s: _rng.normal(s) * 0.05)(B, Hkv, Sk, Dh)),
            "v_cache": _w((lambda *s: _rng.normal(s) * 0.05)(B, Hkv, Sk, Dh)),
            "wq": _w((lambda *s: _rng.normal(s) * 0.05)(D, Hq * Dh) * (D ** -0.5)),
            "wo": _w((lambda *s: _rng.normal(s) * 0.05)(Hq * Dh, D) * ((Hq * Dh) ** -0.5)),
        }
    _A_in = _A_setup()

    def _B_setup():
        B, S, D, F, C = 1, 1, 512, 1376, 1
        return {
            "x": _w((lambda *s: _rng.normal(s) * 0.05)(B, S, D)),
            "w_r": _w((lambda *s: _rng.normal(s) * 0.05)(D)),
            "w_gate": _w((lambda *s: _rng.normal(s) * 0.05)(D, F)),
            "w_up": _w((lambda *s: _rng.normal(s) * 0.05)(D, F)),
            "w_down": _w((lambda *s: _rng.normal(s) * 0.05)(F, D)),
        }
    _B_in = _B_setup()

    return {
        "A_x": _A_in["x"],
        "A_k_cache": _A_in["k_cache"],
        "A_v_cache": _A_in["v_cache"],
        "A_wq": _A_in["wq"],
        "A_wo": _A_in["wo"],
        "B_x": _B_in["x"],
        "B_w_r": _B_in["w_r"],
        "B_w_gate": _B_in["w_gate"],
        "B_w_up": _B_in["w_up"],
        "B_w_down": _B_in["w_down"],
    }

def reference(A_x, A_k_cache, A_v_cache, A_wq, A_wo, B_x, B_w_r, B_w_gate, B_w_up, B_w_down):
    def _A_ref(x, k_cache, v_cache, wq, wo):
        B, Sq, D = x.shape
        Hq, Dh = 32, 128
        Hkv, Sk = k_cache.shape[1], k_cache.shape[2]
        W = min(4096, max(256, Sk // 4))
        rep = Hq // Hkv
        q = (lambda x, *d: x.transpose(*d))((x @ wq).reshape(B, Sq, Hq, Dh), 0, 2, 1, 3)
        k = jnp.repeat(k_cache[:, :, Sk - W:, :], rep, axis=1)
        v = jnp.repeat(v_cache[:, :, Sk - W:, :], rep, axis=1)
        scores = jnp.einsum("bhqd,bhkd->bhqk", q, k) * (Dh ** -0.5)
        p = _softmax(scores, axis=-1)
        o = jnp.einsum("bhqk,bhkd->bhqd", p, v)
        return (lambda x, *d: x.transpose(*d))(o, 0, 2, 1, 3).reshape(B, Sq, Hq * Dh) @ wo

    def _B_ref(x, w_r, w_gate, w_up, w_down):
        B, S, D = x.shape
        C = 1
        r = x @ w_r
        idx = jnp.argsort(-r, axis=-1)[:, :C]
        idx_e = jnp.repeat(idx.reshape(B, C, 1), D, axis=2)
        x_sel = jnp.take_along_axis(x, idx_e, axis=1)
        g = _silu(x_sel @ w_gate)
        u = x_sel @ w_up
        y = (g * u) @ w_down
        r_sel = _sigmoid(jnp.take_along_axis(r, idx, axis=1))
        y = y * r_sel.reshape(B, C, 1)
        b_off = (jnp.arange(B) * S).reshape(B, 1)
        flat_idx = (idx + b_off).reshape(B * C)
        zero = (x * 0.0).reshape(B * S, D)
        upd = _scatter_add(zero, flat_idx, y.reshape(B * C, D), axis=0)
        return x + upd.reshape(B, S, D)

    x = A_x
    xn = _layernorm(x, axis=-1)
    s = _A_ref(xn, A_k_cache, A_v_cache, A_wq, A_wo)
    g = _silu(_B_ref(xn, B_w_r, B_w_gate, B_w_up, B_w_down))
    return x + s * g
```

```python
import functools
import jax
import jax.numpy as jnp
from jax.experimental import pallas as pl
from jax.experimental.pallas import tpu as pltpu

H, DH, W, D, F = 32, 128, 4096, 512, 1376
EPS = 1e-5
NT = (((1,), (1,)), ((), ()))


def make(chunk=128, nbuf=3, compute=True, hpi=1):
    per = W // chunk

    def kern(x_hbm, k_hbm, v_hbm, wq_hbm, wo_hbm, wr_hbm, wg_hbm, wu_hbm, wd_hbm,
             o_ref,
             x_buf, wr_buf, wq_buf, wo_buf, wg_buf, wu_buf, wd_buf,
             kb, vb, q_scr, p_scr, sem_small, sem_w, sem_k, sem_v):
        S = k_hbm.shape[2]
        S0 = S - W

        def k_chunk(h, slot, c):
            return pltpu.make_async_copy(k_hbm.at[0, h, pl.ds(S0 + c * chunk, chunk), :],
                                         kb.at[slot, pl.ds(c * chunk, chunk)], sem_k.at[slot])

        def v_chunk(h, slot, c):
            return pltpu.make_async_copy(v_hbm.at[0, h, pl.ds(S0 + c * chunk, chunk), :],
                                         vb.at[slot, pl.ds(c * chunk, chunk)], sem_v.at[slot])

        def start_k(h, slot):
            for c in range(per):
                k_chunk(h, slot, c).start(priority=c % 2)

        def start_v(h, slot):
            for c in range(per):
                v_chunk(h, slot, c).start(priority=c % 2)

        def start_kv(hk, hv, slot):
            for c in range(0, per, 2):
                k_chunk(hk, slot, c).start(priority=0)
                k_chunk(hk, slot, c + 1).start(priority=1)
                v_chunk(hv, slot, c).start(priority=0)
                v_chunk(hv, slot, c + 1).start(priority=1)

        def wait_k(slot):
            pltpu.make_async_copy(kb.at[slot], kb.at[slot], sem_k.at[slot]).wait()

        def wait_v(slot):
            pltpu.make_async_copy(vb.at[slot], vb.at[slot], sem_v.at[slot]).wait()

        cx = pltpu.make_async_copy(x_hbm, x_buf, sem_small.at[0])
        cr = pltpu.make_async_copy(wr_hbm, wr_buf, sem_small.at[1])
        cx.start()
        cr.start(priority=1)
        i = 0
        for r in range(0, D, 16):
            for c in range(0, H * DH, 1024):
                pltpu.make_async_copy(wq_hbm.at[pl.ds(r, 16), pl.ds(c, 1024)],
                                      wq_buf.at[pl.ds(r, 16), pl.ds(c, 1024)],
                                      sem_w.at[0]).start(priority=i % 2)
                i += 1
        start_k(0, nbuf - 1)
        for src, dst, si in ((wg_hbm, wg_buf, 1), (wu_hbm, wu_buf, 2)):
            for j, r in enumerate(range(0, F, 32)):
                pltpu.make_async_copy(src.at[pl.ds(r, 32), :], dst.at[pl.ds(r, 32), :],
                                      sem_w.at[si]).start(priority=j % 2)
        for j, r in enumerate(range(0, F, 32)):
            pltpu.make_async_copy(wd_hbm.at[pl.ds(r, 32), :], wd_buf.at[pl.ds(r, 32), :],
                                  sem_w.at[3]).start(priority=j % 2)
        for j, r in enumerate(range(0, H * DH, 32)):
            pltpu.make_async_copy(wo_hbm.at[pl.ds(r, 32), :], wo_buf.at[pl.ds(r, 32), :],
                                  sem_w.at[4]).start(priority=j % 2)
        for g in range(nbuf - 2):
            start_kv(g + 1, g, g)

        cx.wait()
        cr.wait()
        x = x_buf[...].reshape(1, D).astype(jnp.float32)
        mu = jnp.mean(x, axis=-1, keepdims=True)
        xc = x - mu
        var = jnp.mean(xc * xc, axis=-1, keepdims=True)
        xn = xc / jnp.sqrt(var + EPS)
        xn_b = xn.astype(jnp.bfloat16)
        r = jnp.sum(xn_b.astype(jnp.float32) * wr_buf[...].reshape(1, D).astype(jnp.float32),
                    axis=-1, keepdims=True)

        pltpu.make_async_copy(wq_buf, wq_buf, sem_w.at[0]).wait()
        if compute:
            q_all = jnp.dot(xn_b, wq_buf[...], preferred_element_type=jnp.float32)
            for h in range(H):
                q_scr[h] = q_all[:, h * DH:(h + 1) * DH]
        scale = DH ** -0.5

        def scores_softmax(h, slot):
            q = q_scr[h].astype(jnp.bfloat16)
            s = jax.lax.dot_general(q, kb[slot], NT, preferred_element_type=jnp.float32)
            m = jnp.max(s, axis=-1, keepdims=True)
            p = jnp.exp((s - m) * scale)
            l = jnp.sum(p, axis=-1, keepdims=True)
            return p, l

        wait_k(nbuf - 1)
        if compute:
            p0, l0 = scores_softmax(0, nbuf - 1)
            p_scr[...] = (p0 * (1.0 / l0)).astype(jnp.bfloat16)
        start_kv(nbuf - 1, nbuf - 2, nbuf - 2)

        pltpu.make_async_copy(wg_buf, wg_buf, sem_w.at[1]).wait()
        pltpu.make_async_copy(wu_buf, wu_buf, sem_w.at[2]).wait()
        pltpu.make_async_copy(wd_buf, wd_buf, sem_w.at[3]).wait()
        if compute:
            gt = jax.lax.dot_general(xn_b, wg_buf[...], NT, preferred_element_type=jnp.float32)
            up = jax.lax.dot_general(xn_b, wu_buf[...], NT, preferred_element_type=jnp.float32)
            hmid = (gt * jax.nn.sigmoid(gt) * up).astype(jnp.bfloat16)
            y = jnp.dot(hmid, wd_buf[...], preferred_element_type=jnp.float32)
            y = y * jax.nn.sigmoid(r)
            bres = xn + (xn * 0.0 + y)
            gate = bres * jax.nn.sigmoid(bres)
        else:
            gate = xn
        pltpu.make_async_copy(wo_buf, wo_buf, sem_w.at[4]).wait()

        def pv_wo(h, slot, acc):
            o = jnp.dot(p_scr[...], vb[slot], preferred_element_type=jnp.float32)
            wo_h = wo_buf[pl.ds(pl.multiple_of(h * DH, DH), DH), :]
            return acc + jnp.dot(o.astype(jnp.bfloat16), wo_h, preferred_element_type=jnp.float32)

        def body(g, acc):
            slot = jax.lax.rem(g, nbuf)
            ng = g + nbuf - 1
            nslot = jax.lax.rem(ng, nbuf)

            @pl.when(ng < H - 1)
            def _():
                start_kv(ng + 1, ng, nslot)

            @pl.when(ng == H - 1)
            def _():
                start_v(ng, nslot)

            wait_k(slot)
            wait_v(slot)
            if compute:
                acc = pv_wo(g, slot, acc)
                p, l = scores_softmax(g + 1, slot)
                p_scr[...] = (p * (1.0 / l)).astype(jnp.bfloat16)
            return acc

        acc = jax.lax.fori_loop(0, H - 1, body, jnp.zeros((1, D), jnp.float32))
        slot = (H - 1) % nbuf
        wait_v(slot)
        if compute:
            acc = pv_wo(H - 1, slot, acc)
        out = x + acc * gate
        o_ref[...] = out.astype(o_ref.dtype).reshape(1, 1, D)

    def fn(A_x, A_k_cache, A_v_cache, A_wq, A_wo, B_x, B_w_r, B_w_gate, B_w_up, B_w_down):
        any_spec = pl.BlockSpec(memory_space=pltpu.HBM)
        bf = jnp.bfloat16
        return pl.pallas_call(
            kern,
            out_shape=jax.ShapeDtypeStruct((1, 1, D), A_x.dtype),
            in_specs=[any_spec] * 9,
            out_specs=pl.BlockSpec(memory_space=pltpu.VMEM),
            scratch_shapes=[
                pltpu.VMEM((1, 1, D), bf), pltpu.VMEM((D,), bf),
                pltpu.VMEM((D, H * DH), bf), pltpu.VMEM((H * DH, D), bf),
                pltpu.VMEM((F, D), bf), pltpu.VMEM((F, D), bf), pltpu.VMEM((F, D), bf),
                pltpu.VMEM((nbuf, W, DH), bf), pltpu.VMEM((nbuf, W, DH), bf),
                pltpu.VMEM((H, 1, DH), jnp.float32), pltpu.VMEM((1, W), bf),
                pltpu.SemaphoreType.DMA((2,)), pltpu.SemaphoreType.DMA((5,)),
                pltpu.SemaphoreType.DMA((nbuf,)), pltpu.SemaphoreType.DMA((nbuf,)),
            ],
            compiler_params=pltpu.CompilerParams(vmem_limit_bytes=64 * 1024 * 1024),
        )(A_x, A_k_cache, A_v_cache, A_wq, A_wo, B_w_r, B_w_gate.T, B_w_up.T, B_w_down)

    return fn


_impl = make(chunk=128, nbuf=3)


@jax.jit
def pallas_recurrent_scan__sliding_block_cached__moe_arch_mod__decode_kernel(
    A_x, A_k_cache, A_v_cache, A_wq, A_wo, B_x, B_w_r, B_w_gate, B_w_up, B_w_down,
):
    return _impl(A_x, A_k_cache, A_v_cache, A_wq, A_wo, B_x, B_w_r, B_w_gate, B_w_up, B_w_down)
```

```python
import functools
import jax
import jax.numpy as jnp
from jax.experimental import pallas as pl
from jax.experimental.pallas import tpu as pltpu

H, DH, W, D, F = 32, 128, 4096, 512, 1376
EPS = 1e-5
NT = (((1,), (1,)), ((), ()))
bf = jnp.bfloat16
f32 = jnp.float32


def zip_pairs(xs, ys):
    out = []
    i = j = 0
    while i < len(xs) or j < len(ys):
        for lst, k in ((xs, i), (ys, j)):
            for t, item in enumerate(lst[k:k + 2]):
                out.append((item, t))
        i += 2
        j += 2
    return out


def halves(xs):
    n = len(xs)
    h = (n // 2 + 1) // 2 * 2
    return zip_pairs(xs[:h], xs[h:])


def make(chunk=128, nbuf=3, compute=True, pattern='p1', wplan='A', nobc=True, nosc=False):
    per = W // chunk

    def kern(x_hbm, k_hbm, v_hbm, wq_hbm, wo_hbm, wr_hbm, wg_hbm, wu_hbm, wd_hbm,
             o_ref,
             x_buf, wr_buf, wq_buf, wo_buf, wg_buf, wu_buf, wd_buf,
             kb, vb, q_scr, p_scr, sems):
        S = k_hbm.shape[2]
        S0 = S - W
        SEM_A = nbuf - 1
        SEM_B = nbuf

        def kv_copy(a, h, slot, c):
            hb, buf = ((k_hbm, kb), (v_hbm, vb))[a]
            return pltpu.make_async_copy(hb.at[0, h, pl.ds(S0 + c * chunk, chunk), :],
                                         buf.at[slot, pl.ds(c * chunk, chunk)], sems.at[slot])

        def kv_seq():
            if pattern == 'p1':
                return [(a, c + t, t) for c in range(0, per, 2) for a in range(2) for t in range(2)]
            if pattern == 'stride2':
                return [(a, c + u + 2 * t, t) for c in range(0, per, 4) for u in range(2) for a in range(2) for t in range(2)]

        def start_kv(hk, hv, slot):
            for a, c, q in kv_seq():
                kv_copy(a, (hk, hv)[a], slot, c).start(priority=q)

        def start_single(a, h, slot):
            for cp, q in halves([kv_copy(a, h, slot, c) for c in range(per)]):
                cp.start(priority=q)

        def wait_full(ref, sem):
            pltpu.make_async_copy(ref, ref, sem).wait()

        def rows32(src, dst, sem, nrows):
            return [pltpu.make_async_copy(src.at[pl.ds(r, 32), :], dst.at[pl.ds(r, 32), :], sem) for r in range(0, nrows, 32)]

        wq_c = [pltpu.make_async_copy(wq_hbm.at[pl.ds(r, 8), pl.ds(c, 2048)], wq_buf.at[pl.ds(r, 8), pl.ds(c, 2048)], sems.at[SEM_A])
                for r in range(0, D, 8) for c in range(0, H * DH, 2048)]
        k0_c = [kv_copy(0, 0, nbuf - 1, c) for c in range(per)]
        wg_c = rows32(wg_hbm, wg_buf, sems.at[SEM_B], F)
        wu_c = rows32(wu_hbm, wu_buf, sems.at[SEM_B], F)
        wd_c = rows32(wd_hbm, wd_buf, sems.at[SEM_B], F)
        wo_c = rows32(wo_hbm, wo_buf, sems.at[SEM_B], H * DH)

        cx = pltpu.make_async_copy(x_hbm, x_buf, sems.at[SEM_A])
        cr = pltpu.make_async_copy(wr_hbm, wr_buf, sems.at[SEM_A])
        cx.start()
        cr.start(priority=1)
        if wplan == 'A':
            prog = halves(wq_c) + zip_pairs(k0_c, wd_c[:32]) + zip_pairs(wg_c, wu_c) + halves(wd_c[32:] ) + halves(wo_c)
        elif wplan == 'B':
            prog = zip_pairs(wq_c, wo_c) + zip_pairs(k0_c, wd_c[:32]) + zip_pairs(wg_c, wu_c) + halves(wd_c[32:])
        elif wplan == 'C':
            allc = wq_c + k0_c + wg_c + wu_c + wd_c + wo_c
            prog = [(c, i % 2) for i, c in enumerate(allc)]
        for cp, q in prog:
            cp.start(priority=q)
        for g in range(nbuf - 2):
            start_kv(g + 1, g, g)

        cx.wait()
        cr.wait()
        wait_full(wq_buf, sems.at[SEM_A])
        wait_full(kb.at[nbuf - 1], sems.at[SEM_A])
        x = x_buf[...].reshape(1, D).astype(f32)
        mu = jnp.mean(x, axis=-1, keepdims=True)
        xc = x - mu
        var = jnp.mean(xc * xc, axis=-1, keepdims=True)
        xn = xc / jnp.sqrt(var + EPS)
        xn_b = xn.astype(bf)
        r = jnp.sum(xn_b.astype(f32) * wr_buf[...].reshape(1, D).astype(f32), axis=-1, keepdims=True)
        scale = DH ** -0.5

        if compute:
            q_all = jnp.dot(xn_b, wq_buf[...], preferred_element_type=f32)
            for h in range(H):
                q_scr[h] = q_all[:, h * DH:(h + 1) * DH]

        def scores_softmax(h, slot):
            q = q_scr[h].astype(bf)
            s = jax.lax.dot_general(q, kb[slot], NT, preferred_element_type=f32)
            m = jnp.max(s, axis=-1, keepdims=True)
            p = jnp.exp((s - m) * scale)
            l = jnp.sum(p, axis=-1, keepdims=True)
            p_scr[...] = (p * (1.0 / l)).astype(bf)

        if compute:
            scores_softmax(0, nbuf - 1)
        start_kv(nbuf - 1, nbuf - 2, nbuf - 2)

        wait_full(wg_buf, sems.at[SEM_B])
        wait_full(wu_buf, sems.at[SEM_B])
        wait_full(wd_buf, sems.at[SEM_B])
        wait_full(wo_buf, sems.at[SEM_B])
        if compute:
            gt = jax.lax.dot_general(xn_b, wg_buf[...], NT, preferred_element_type=f32)
            up = jax.lax.dot_general(xn_b, wu_buf[...], NT, preferred_element_type=f32)
            hmid = (gt * jax.nn.sigmoid(gt) * up).astype(bf)
            y = jnp.dot(hmid, wd_buf[...], preferred_element_type=f32)
            y = y * jax.nn.sigmoid(r)
            bres = xn + (xn * 0.0 + y)
            gate = bres * jax.nn.sigmoid(bres)
        else:
            gate = xn

        def pv_wo(h, slot, acc):
            o = jnp.dot(p_scr[...], vb[slot], preferred_element_type=f32)
            wo_h = wo_buf[pl.ds(pl.multiple_of(h * DH, DH), DH), :]
            return acc + jnp.dot(o.astype(bf), wo_h, preferred_element_type=f32)

        def body(g, acc):
            slot = jax.lax.rem(g, nbuf)
            ng = g + nbuf - 1
            nslot = jax.lax.rem(ng, nbuf)

            @pl.when(ng < H - 1)
            def _():
                start_kv(ng + 1, ng, nslot)

            @pl.when(ng == H - 1)
            def _():
                start_single(1, ng, nslot)

            wait_full(kb.at[slot], sems.at[slot])
            wait_full(vb.at[slot], sems.at[slot])
            if compute:
                acc = pv_wo(g, slot, acc)
                scores_softmax(g + 1, slot)
            return acc

        acc = jax.lax.fori_loop(0, H - 1, body, jnp.zeros((1, D), f32))
        slot = (H - 1) % nbuf
        wait_full(vb.at[slot], sems.at[slot])
        if compute:
            acc = pv_wo(H - 1, slot, acc)
        out = x + acc * gate
        o_ref[...] = out.astype(o_ref.dtype).reshape(1, 1, D)

    def fn(A_x, A_k_cache, A_v_cache, A_wq, A_wo, B_x, B_w_r, B_w_gate, B_w_up, B_w_down):
        hbm = pl.BlockSpec(memory_space=pltpu.HBM)
        return pl.pallas_call(
            kern,
            out_shape=jax.ShapeDtypeStruct((1, 1, D), A_x.dtype),
            in_specs=[hbm] * 9,
            out_specs=pl.BlockSpec(memory_space=pltpu.VMEM),
            scratch_shapes=[
                pltpu.VMEM((1, 1, D), bf), pltpu.VMEM((D,), bf),
                pltpu.VMEM((D, H * DH), bf), pltpu.VMEM((H * DH, D), bf),
                pltpu.VMEM((F, D), bf), pltpu.VMEM((F, D), bf), pltpu.VMEM((F, D), bf),
                pltpu.VMEM((nbuf, W, DH), bf), pltpu.VMEM((nbuf, W, DH), bf),
                pltpu.VMEM((H, 1, DH), f32), pltpu.VMEM((1, W), bf),
                pltpu.SemaphoreType.DMA((nbuf + 1,)),
            ],
            compiler_params=pltpu.CompilerParams(vmem_limit_bytes=64 * 1024 * 1024, disable_bounds_checks=nobc,
                                                 disable_semaphore_checks=nosc),
        )(A_x, A_k_cache, A_v_cache, A_wq, A_wo, B_w_r, B_w_gate.T, B_w_up.T, B_w_down)

    return fn


_impl = make()


@jax.jit
def pallas_recurrent_scan__sliding_block_cached__moe_arch_mod__decode_kernel(
    A_x, A_k_cache, A_v_cache, A_wq, A_wo, B_x, B_w_r, B_w_gate, B_w_up, B_w_down,
):
    return _impl(A_x, A_k_cache, A_v_cache, A_wq, A_wo, B_x, B_w_r, B_w_gate, B_w_up, B_w_down)
```

```python
import contextlib
import jax
import jax.numpy as jnp
from jax.experimental import pallas as pl
from jax.experimental.pallas import tpu as pltpu

def spairs(xs, s):
    n = len(xs)
    l0 = [c for c in range(n) if (c // s) % 2 == 0]
    l1 = [c for c in range(n) if (c // s) % 2 == 1]
    m = min(len(l0), len(l1))
    pairs = [(xs[a], xs[b]) for a, b in zip(l0[:m], l1[:m])]
    rest = l0[m:] + l1[m:]
    for i in range(0, len(rest), 2):
        pairs.append(tuple(xs[c] for c in rest[i:i + 2]))
    return pairs


def alternate(px, py):
    out = []
    for i in range(max(len(px), len(py))):
        if i < len(px): out.append(px[i])
        if i < len(py): out.append(py[i])
    return out


def two(xs, ys, s):
    return alternate(spairs(xs, s), spairs(ys, s))


def one(xs, s):
    h = (len(xs) // 2 + 1) // 2 * 2
    return two(xs[:h], xs[h:], s)


def issue(pairs):
    for p in pairs:
        for q, cp in enumerate(p):
            cp.start(priority=q)


H, DH, W, D, F = 32, 128, 4096, 512, 1376
EPS = 1e-5
NT = (((1,), (1,)), ((), ()))
bf = jnp.bfloat16
f32 = jnp.float32


def make(chunk=128, nbuf=3, compute=True, s=8, L=3, vsplit=(16,), scopes=False, name=None):
    per = W // chunk
    scope = jax.named_scope if scopes else (lambda n: contextlib.nullcontext())
    NP = L + 1

    def kern(x_hbm, k_hbm, v_hbm, wq_hbm, wo_hbm, wr_hbm, wg_hbm, wu_hbm, wd_hbm,
             o_ref,
             x_buf, wr_buf, wq_buf, wo_buf, wg_buf, wu_buf, wd_buf,
             k0b, kb, vb, q_scr, p_scr, sems):
        S = k_hbm.shape[2]
        S0 = S - W
        SEM_A = nbuf
        SEM_B = nbuf + 1

        def cp(hb, h, dst, c, sem):
            return pltpu.make_async_copy(hb.at[0, h, pl.ds(S0 + c * chunk, chunk), :], dst.at[pl.ds(c * chunk, chunk)], sem)

        def k_list(h, slot):
            return [cp(k_hbm, h, kb.at[slot], c, sems.at[slot]) for c in range(per)]

        def v_list(h, slot, sem=None, lo=0, hi=per):
            return [cp(v_hbm, h, vb.at[slot], c, sems.at[slot] if sem is None else sem) for c in range(lo, hi)]

        def wait_full(ref, sem):
            pltpu.make_async_copy(ref, ref, sem).wait()

        def rows32(src, dst, sem, nrows):
            return [pltpu.make_async_copy(src.at[pl.ds(r, 32), :], dst.at[pl.ds(r, 32), :], sem) for r in range(0, nrows, 32)]

        wq_c = [pltpu.make_async_copy(wq_hbm.at[pl.ds(r, 8), pl.ds(c, 2048)], wq_buf.at[pl.ds(r, 8), pl.ds(c, 2048)], sems.at[SEM_A])
                for r in range(0, D, 8) for c in range(0, H * DH, 2048)]
        kinit = [[cp(k_hbm, j, k0b.at[j], c, sems.at[SEM_A]) for c in range(per)] for j in range(L)]
        wg_c = rows32(wg_hbm, wg_buf, sems.at[SEM_B], F)
        wu_c = rows32(wu_hbm, wu_buf, sems.at[SEM_B], F)
        wd_c = rows32(wd_hbm, wd_buf, sems.at[SEM_B], F)
        wo_c = rows32(wo_hbm, wo_buf, sems.at[SEM_B], H * DH)

        cx = pltpu.make_async_copy(x_hbm, x_buf, sems.at[SEM_A])
        cr = pltpu.make_async_copy(wr_hbm, wr_buf, sems.at[SEM_A])
        prog = [(cx, cr)] + two(wq_c, wo_c, s)
        for j in range(0, L - 1, 2):
            prog += two(kinit[j], kinit[j + 1], s)
        if L % 2:
            prog += two(kinit[L - 1], wd_c[:32], s) + two(wg_c, wu_c, s) + one(wd_c[32:], s)
        else:
            prog += two(wg_c, wu_c, s) + one(wd_c, s)
        issue(prog)
        for g in range(nbuf - 2):
            issue(two(k_list(g + L, g), v_list(g, g), s))

        cx.wait()
        cr.wait()
        wait_full(wq_buf, sems.at[SEM_A])
        wait_full(k0b, sems.at[SEM_A])
        x = x_buf[...].reshape(1, D).astype(f32)
        mu = jnp.mean(x, axis=-1, keepdims=True)
        xc = x - mu
        var = jnp.mean(xc * xc, axis=-1, keepdims=True)
        xn = xc / jnp.sqrt(var + EPS)
        xn_b = xn.astype(bf)
        r = jnp.sum(xn_b.astype(f32) * wr_buf[...].reshape(1, D).astype(f32), axis=-1, keepdims=True)
        scale = DH ** -0.5

        if compute:
            q_all = jnp.dot(xn_b, wq_buf[...], preferred_element_type=f32)
            for h in range(H):
                q_scr[h] = q_all[:, h * DH:(h + 1) * DH]

        def scores_softmax(h, kref, pslot):
            q = q_scr[h].astype(bf)
            s_ = jax.lax.dot_general(q, kref[...], NT, preferred_element_type=f32)
            m = jnp.max(s_, axis=-1, keepdims=True)
            p = jnp.exp((s_ - m) * scale)
            l = jnp.sum(p, axis=-1, keepdims=True)
            p_scr[pslot] = (p * (1.0 / l)).astype(bf)

        if compute:
            def init_body(j, _):
                scores_softmax(j, k0b.at[j], j)
            jax.lax.fori_loop(0, L, init_body, None)
        issue(two(k_list(nbuf - 2 + L, nbuf - 2), v_list(nbuf - 2, nbuf - 2), s))

        wait_full(wg_buf, sems.at[SEM_B])
        wait_full(wu_buf, sems.at[SEM_B])
        wait_full(wd_buf, sems.at[SEM_B])
        wait_full(wo_buf, sems.at[SEM_B])
        if compute:
            gt = jax.lax.dot_general(xn_b, wg_buf[...], NT, preferred_element_type=f32)
            up = jax.lax.dot_general(xn_b, wu_buf[...], NT, preferred_element_type=f32)
            hmid = (gt * jax.nn.sigmoid(gt) * up).astype(bf)
            y = jnp.dot(hmid, wd_buf[...], preferred_element_type=f32)
            y = y * jax.nn.sigmoid(r)
            bres = xn + (xn * 0.0 + y)
            gate = bres * jax.nn.sigmoid(bres)
        else:
            gate = xn

        def pv_wo(h, slot, pslot, acc):
            o = jnp.dot(p_scr[pslot], vb[slot], preferred_element_type=f32)
            wo_h = wo_buf[pl.ds(pl.multiple_of(h * DH, DH), DH), :]
            return acc + jnp.dot(o.astype(bf), wo_h, preferred_element_type=f32)

        bounds = [0] + list(vsplit) + [per]
        last_slot = (H - 1) % nbuf
        piece_sems = [last_slot, SEM_A, SEM_B]
        assert len(bounds) - 1 <= 3

        def prefetch(g):
            ng = g + nbuf - 1
            nslot = jax.lax.rem(ng, nbuf)

            @pl.when(ng < H - L)
            def _():
                issue(two(k_list(ng + L, nslot), v_list(ng, nslot), s))

            @pl.when((ng >= H - L) & (ng < H - 1))
            def _():
                issue(one(v_list(ng, nslot), s))

            @pl.when(ng == H - 1)
            def _():
                for i in range(len(bounds) - 1):
                    issue(one(v_list(H - 1, last_slot, sems.at[piece_sems[i]], bounds[i], bounds[i + 1]), s))

        def body(g, acc):
            slot = jax.lax.rem(g, nbuf)
            prefetch(g)
            with scope("it_wait"):
                wait_full(kb.at[slot], sems.at[slot])
                wait_full(vb.at[slot], sems.at[slot])
            with scope("it_comp"):
                if compute:
                    acc = pv_wo(g, slot, jax.lax.rem(g, NP), acc)
                    scores_softmax(g + L, kb.at[slot], jax.lax.rem(g + L, NP))
            return acc

        def body2(g, acc):
            slot = jax.lax.rem(g, nbuf)
            prefetch(g)
            with scope("it2_wait"):
                wait_full(vb.at[slot], sems.at[slot])
            with scope("it2_comp"):
                if compute:
                    acc = pv_wo(g, slot, jax.lax.rem(g, NP), acc)
            return acc

        acc = jax.lax.fori_loop(0, H - L, body, jnp.zeros((1, D), f32))
        acc = jax.lax.fori_loop(H - L, H - 1, body2, acc)
        o = None
        ps = (H - 1) % NP
        for i in range(len(bounds) - 1):
            r0, r1 = bounds[i] * chunk, bounds[i + 1] * chunk
            with scope(f"e_wait31_{i}"):
                wait_full(vb.at[last_slot, pl.ds(r0, r1 - r0)], sems.at[piece_sems[i]])
            with scope(f"e_pv31_{i}"):
                if compute:
                    oi = jnp.dot(p_scr[ps, :, r0:r1], vb[last_slot, r0:r1, :], preferred_element_type=f32)
                    o = oi if o is None else o + oi
        with scope("e_wo"):
            if compute:
                acc = acc + jnp.dot(o.astype(bf), wo_buf[(H - 1) * DH:H * DH, :], preferred_element_type=f32)
        out = x + acc * gate
        o_ref[...] = out.astype(o_ref.dtype).reshape(1, 1, D)

    def fn(A_x, A_k_cache, A_v_cache, A_wq, A_wo, B_x, B_w_r, B_w_gate, B_w_up, B_w_down):
        hbm = pl.BlockSpec(memory_space=pltpu.HBM)
        return pl.pallas_call(
            kern,
            out_shape=jax.ShapeDtypeStruct((1, 1, D), A_x.dtype),
            in_specs=[hbm] * 9,
            out_specs=pl.BlockSpec(memory_space=pltpu.VMEM),
            scratch_shapes=[
                pltpu.VMEM((1, 1, D), bf), pltpu.VMEM((D,), bf),
                pltpu.VMEM((D, H * DH), bf), pltpu.VMEM((H * DH, D), bf),
                pltpu.VMEM((F, D), bf), pltpu.VMEM((F, D), bf), pltpu.VMEM((F, D), bf),
                pltpu.VMEM((L, W, DH), bf), pltpu.VMEM((nbuf, W, DH), bf), pltpu.VMEM((nbuf, W, DH), bf),
                pltpu.VMEM((H, 1, DH), f32), pltpu.VMEM((NP, 1, W), bf),
                pltpu.SemaphoreType.DMA((nbuf + 2,)),
            ],
            name=name,
            compiler_params=pltpu.CompilerParams(vmem_limit_bytes=64 * 1024 * 1024, disable_bounds_checks=True),
        )(A_x, A_k_cache, A_v_cache, A_wq, A_wo, B_w_r, B_w_gate.T, B_w_up.T, B_w_down)

    return fn


_impl = make(L=3, vsplit=())


@jax.jit
def pallas_recurrent_scan__sliding_block_cached__moe_arch_mod__decode_kernel(
    A_x, A_k_cache, A_v_cache, A_wq, A_wo, B_x, B_w_r, B_w_gate, B_w_up, B_w_down,
):
    return _impl(A_x, A_k_cache, A_v_cache, A_wq, A_wo, B_x, B_w_r, B_w_gate, B_w_up, B_w_down)
```

```python
import jax
import jax.numpy as jnp
from jax.experimental import pallas as pl
from jax.experimental.pallas import tpu as pltpu

H, DH, D, F = 32, 128, 512, 1376
EPS = 1e-5
NT = (((1,), (1,)), ((), ()))
BF = jnp.bfloat16
F32 = jnp.float32

CHUNK = 128
WROWS = 32
STRIDE = 8
NBUF = 3
LEAD = 2
K_SKEW = 0
V_SKEW = 64


def _pairs(xs, s=STRIDE):
    n = len(xs)
    l0 = [c for c in range(n) if (c // s) % 2 == 0]
    l1 = [c for c in range(n) if (c // s) % 2 == 1]
    m = min(len(l0), len(l1))
    out = [(xs[a], xs[b]) for a, b in zip(l0, l1)]
    rest = [xs[c] for c in l0[m:] + l1[m:]]
    out += [tuple(rest[i:i + 2]) for i in range(0, len(rest), 2)]
    return out


def _two(xs, ys):
    px, py = _pairs(xs), _pairs(ys)
    out = []
    for i in range(max(len(px), len(py))):
        out += px[i:i + 1] + py[i:i + 1]
    return out


def _one(xs):
    h = (len(xs) // 2 + 1) // 2 * 2
    return _two(xs[:h], xs[h:])


def _issue(pairs):
    for p in pairs:
        for queue, copy in enumerate(p):
            copy.start(priority=queue)


def _chunks(rows, skew):
    b = [0] + list(range(skew if skew else CHUNK, rows, CHUNK)) + [rows]
    pieces = [(b[i], b[i + 1] - b[i]) for i in range(len(b) - 1)]
    return pieces if not skew else pieces[1:-1] + [pieces[0], pieces[-1]]


def make(k_skew=K_SKEW, v_skew=V_SKEW, nobc=True, name=None):
    def kernel(x_hbm, k_hbm, v_hbm, wq_hbm, wo_hbm, wr_hbm, wg_hbm, wu_hbm, wd_hbm,
               o_ref,
               x_buf, wr_buf, wq_buf, wo_buf, wg_buf, wu_buf, wd_buf,
               k0_buf, k_buf, v_buf, q_scr, p_scr, sems):
        seq = k_hbm.shape[2]
        win = k_buf.shape[1]
        s0 = seq - win
        sem_a, sem_b = sems.at[NBUF], sems.at[NBUF + 1]
        k_pieces, v_pieces = _chunks(win, k_skew), _chunks(win, v_skew)
        n_p = LEAD + 1

        def head_copies(hbm, h, dst, pieces, sem):
            return [pltpu.make_async_copy(hbm.at[0, h, pl.ds(s0 + r, n), :], dst.at[pl.ds(r, n)], sem)
                    for r, n in pieces]

        def row_copies(src, dst, sem, lo, hi):
            return [pltpu.make_async_copy(src.at[pl.ds(r, WROWS), :], dst.at[pl.ds(r, WROWS), :], sem)
                    for r in range(lo, hi, WROWS)]

        def wait_all(buf, sem):
            pltpu.make_async_copy(buf, buf, sem).wait()

        def start_group(g, slot, with_k=True):
            sem = sems.at[slot]
            vs = head_copies(v_hbm, g, v_buf.at[slot], v_pieces, sem)
            if with_k:
                _issue(_two(head_copies(k_hbm, g + LEAD, k_buf.at[slot], k_pieces, sem), vs))
            else:
                _issue(_one(vs))

        cx = pltpu.make_async_copy(x_hbm, x_buf, sem_a)
        cr = pltpu.make_async_copy(wr_hbm, wr_buf, sem_a)
        wq_c = [pltpu.make_async_copy(wq_hbm.at[pl.ds(r, 8), pl.ds(c, 2048)],
                                      wq_buf.at[pl.ds(r, 8), pl.ds(c, 2048)], sem_a)
                for r in range(0, D, 8) for c in range(0, H * DH, 2048)]
        k0_c = [head_copies(k_hbm, j, k0_buf.at[j], k_pieces, sem_a) for j in range(LEAD)]
        wo_early = (H - LEAD) * DH
        _issue([(cx, cr)]
               + _two(wq_c, row_copies(wo_hbm, wo_buf, sem_b, 0, wo_early))
               + _two(k0_c[0], k0_c[1])
               + _two(row_copies(wg_hbm, wg_buf, sem_b, 0, F), row_copies(wu_hbm, wu_buf, sem_b, 0, F))
               + _one(row_copies(wd_hbm, wd_buf, sem_b, 0, F)))
        for g in range(NBUF - 2):
            start_group(g, g)

        cx.wait()
        cr.wait()
        wait_all(wq_buf, sem_a)
        wait_all(k0_buf, sem_a)
        x = x_buf[...].reshape(1, D).astype(F32)
        mu = jnp.mean(x, axis=-1, keepdims=True)
        xc = x - mu
        var = jnp.mean(xc * xc, axis=-1, keepdims=True)
        xn = xc / jnp.sqrt(var + EPS)
        xn_b = xn.astype(BF)
        router = jnp.sum(xn_b.astype(F32) * wr_buf[...].reshape(1, D).astype(F32), axis=-1, keepdims=True)

        q_all = jnp.dot(xn_b, wq_buf[...], preferred_element_type=F32)
        for h in range(H):
            q_scr[h] = q_all[:, h * DH:(h + 1) * DH]

        def scores_softmax(h, k_ref, p_slot):
            q = q_scr[h].astype(BF)
            s = jax.lax.dot_general(q, k_ref[...], NT, preferred_element_type=F32) * (DH ** -0.5)
            e = jnp.exp(s - jnp.max(s, axis=-1, keepdims=True))
            p_scr[p_slot] = (e * (1.0 / jnp.sum(e, axis=-1, keepdims=True))).astype(BF)

        def init_body(j, carry):
            scores_softmax(j, k0_buf.at[j], j)
            return carry

        jax.lax.fori_loop(0, LEAD, init_body, 0)
        start_group(NBUF - 2, NBUF - 2)

        wait_all(wg_buf, sem_b)
        wait_all(wu_buf, sem_b)
        wait_all(wd_buf, sem_b)
        wait_all(wo_buf.at[pl.ds(0, wo_early)], sem_b)
        gt = jax.lax.dot_general(xn_b, wg_buf[...], NT, preferred_element_type=F32)
        up = jax.lax.dot_general(xn_b, wu_buf[...], NT, preferred_element_type=F32)
        y = jnp.dot((gt * jax.nn.sigmoid(gt) * up).astype(BF), wd_buf[...], preferred_element_type=F32)
        routed = xn + (xn * 0.0 + y * jax.nn.sigmoid(router))
        gate = routed * jax.nn.sigmoid(routed)

        def p_times_v(slot, p_slot):
            return jnp.dot(p_scr[p_slot], v_buf[slot], preferred_element_type=F32).astype(BF)

        def body(g, acc):
            ng = g + NBUF - 1
            nslot = jax.lax.rem(ng, NBUF)

            @pl.when(ng < H - LEAD)
            def _():
                start_group(ng, nslot)

            @pl.when(ng >= H - LEAD)
            def _():
                start_group(ng, nslot, with_k=False)

            @pl.when(ng == H - 1)
            def _():
                _issue(_pairs(row_copies(wo_hbm, wo_buf, sem_b, wo_early, H * DH), 2))

            slot = jax.lax.rem(g, NBUF)
            wait_all(k_buf.at[slot], sems.at[slot])
            wait_all(v_buf.at[slot], sems.at[slot])
            wo_h = wo_buf[pl.ds(pl.multiple_of(g * DH, DH), DH), :]
            acc = acc + jnp.dot(p_times_v(slot, jax.lax.rem(g, n_p)), wo_h, preferred_element_type=F32)
            scores_softmax(g + LEAD, k_buf.at[slot], jax.lax.rem(g + LEAD, n_p))
            return acc

        acc = jax.lax.fori_loop(0, H - LEAD, body, jnp.zeros((1, D), F32))

        outs = []
        for g in range(H - LEAD, H):
            wait_all(v_buf.at[g % NBUF], sems.at[g % NBUF])
            outs.append(p_times_v(g % NBUF, g % n_p))
        wait_all(wo_buf.at[pl.ds(wo_early, LEAD * DH)], sem_b)
        for g, o in zip(range(H - LEAD, H), outs):
            acc = acc + jnp.dot(o, wo_buf[g * DH:(g + 1) * DH, :], preferred_element_type=F32)
        o_ref[...] = (x + acc * gate).astype(o_ref.dtype).reshape(1, 1, D)

    def fn(A_x, A_k_cache, A_v_cache, A_wq, A_wo, B_x, B_w_r, B_w_gate, B_w_up, B_w_down):
        del B_x
        win = min(4096, max(256, A_k_cache.shape[2] // 4))
        hbm = pl.BlockSpec(memory_space=pltpu.HBM)
        return pl.pallas_call(
            kernel,
            out_shape=jax.ShapeDtypeStruct((1, 1, D), A_x.dtype),
            in_specs=[hbm] * 9,
            out_specs=pl.BlockSpec(memory_space=pltpu.VMEM),
            scratch_shapes=[
                pltpu.VMEM((1, 1, D), BF), pltpu.VMEM((D,), BF),
                pltpu.VMEM((D, H * DH), BF), pltpu.VMEM((H * DH, D), BF),
                pltpu.VMEM((F, D), BF), pltpu.VMEM((F, D), BF), pltpu.VMEM((F, D), BF),
                pltpu.VMEM((LEAD, win, DH), BF), pltpu.VMEM((NBUF, win, DH), BF), pltpu.VMEM((NBUF, win, DH), BF),
                pltpu.VMEM((H, 1, DH), F32), pltpu.VMEM((LEAD + 1, 1, win), BF),
                pltpu.SemaphoreType.DMA((NBUF + 2,)),
            ],
            name=name,
            compiler_params=pltpu.CompilerParams(vmem_limit_bytes=64 * 1024 * 1024, disable_bounds_checks=nobc),
        )(A_x, A_k_cache, A_v_cache, A_wq, A_wo, B_w_r, B_w_gate.T, B_w_up.T, B_w_down)

    return fn


_impl = make(nobc=False)


@jax.jit
def pallas_recurrent_scan__sliding_block_cached__moe_arch_mod__decode_kernel(
    A_x, A_k_cache, A_v_cache, A_wq, A_wo, B_x, B_w_r, B_w_gate, B_w_up, B_w_down,
):
    return _impl(A_x, A_k_cache, A_v_cache, A_wq, A_wo, B_x, B_w_r, B_w_gate, B_w_up, B_w_down)
```

```python
import jax
import jax.numpy as jnp
from jax.experimental import pallas as pl
from jax.experimental.pallas import tpu as pltpu

H, DH, D, F = 32, 128, 512, 1376
EPS = 1e-5
NT = (((1,), (1,)), ((), ()))
BF = jnp.bfloat16
F32 = jnp.float32

CHUNK = 128
WROWS = 32
STRIDE = 8
NBUF = 3
LEAD = 2
BIG = 256
K_ALIGN = 128
V_ALIGN = 64


def _pairs(xs, s=STRIDE):
    n = len(xs)
    l0 = [c for c in range(n) if (c // s) % 2 == 0]
    l1 = [c for c in range(n) if (c // s) % 2 == 1]
    m = min(len(l0), len(l1))
    out = [(xs[a], xs[b]) for a, b in zip(l0, l1)]
    rest = [xs[c] for c in l0[m:] + l1[m:]]
    out += [tuple(rest[i:i + 2]) for i in range(0, len(rest), 2)]
    return out


def _two(xs, ys):
    px, py = _pairs(xs), _pairs(ys)
    out = []
    for i in range(max(len(px), len(py))):
        out += px[i:i + 1] + py[i:i + 1]
    return out


def _one(xs):
    h = (len(xs) // 2 + 1) // 2 * 2
    return _two(xs[:h], xs[h:])


def _issue(pairs):
    for p in pairs:
        for queue, copy in enumerate(p):
            copy.start(priority=queue)


def _grid(lo, hi, t, step):
    first = lo + (t - lo) % step
    cuts = sorted(set([lo, hi] + list(range(first, hi, step))))
    return [(cuts[i], cuts[i + 1] - cuts[i]) for i in range(len(cuts) - 1)]


def _split(rows, t, n_big, skip):
    lo = t % BIG + skip * BIG
    hi = lo + n_big * BIG
    assert hi <= rows
    return _grid(0, lo, t, CHUNK) + _grid(hi, rows, t, CHUNK), _grid(lo, hi, t, BIG)


def _merge(q0, q1):
    out, i, j = [], 0, 0
    while i < len(q0) or j < len(q1):
        if j >= len(q1) or (i < len(q0) and i * len(q1) <= j * len(q0)):
            out.append((q0[i], 0)); i += 1
        else:
            out.append((q1[j], 1)); j += 1
    return out


def _zip_streams(*lists):
    out = []
    for i in range(max(len(l) for l in lists)):
        out += [l[i] for l in lists if i < len(l)]
    return out


def _start(seq):
    for copy, queue in seq:
        copy.start(priority=queue)


def make(tk=K_ALIGN, tv=V_ALIGN, n_big=11, skip=4, nobc=True, name=None):
    def kernel(x_hbm, k_hbm, v_hbm, wq_hbm, wo_hbm, wr_hbm, wg_hbm, wu_hbm, wd_hbm,
               o_ref,
               x_buf, wr_buf, wq_buf, wo_buf, wg_buf, wu_buf, wd_buf,
               k0_buf, k_buf, v_buf, q_scr, p_scr, sems):
        seq = k_hbm.shape[2]
        win = k_buf.shape[1]
        s0 = seq - win
        sem_a, sem_b = sems.at[NBUF], sems.at[NBUF + 1]
        k_small, k_big = _split(win, tk, n_big, skip)
        v_small, v_big = _split(win, tv, n_big, skip)
        n_p = LEAD + 1

        def head_copies(hbm, h, dst, pieces, sem):
            return [pltpu.make_async_copy(hbm.at[0, h, pl.ds(s0 + r, n), :], dst.at[pl.ds(r, n)], sem)
                    for r, n in pieces]

        def row_copies(src, dst, sem, lo, hi):
            return [pltpu.make_async_copy(src.at[pl.ds(r, WROWS), :], dst.at[pl.ds(r, WROWS), :], sem)
                    for r in range(lo, hi, WROWS)]

        def wait_all(buf, sem):
            pltpu.make_async_copy(buf, buf, sem).wait()

        def start_group(g, slot, with_k=True):
            sem = sems.at[slot]
            v0 = head_copies(v_hbm, g, v_buf.at[slot], v_small, sem)
            v1 = head_copies(v_hbm, g, v_buf.at[slot], v_big, sem)
            if with_k:
                k0 = head_copies(k_hbm, g + LEAD, k_buf.at[slot], k_small, sem)
                k1 = head_copies(k_hbm, g + LEAD, k_buf.at[slot], k_big, sem)
                _start(_merge(_zip_streams(k0, v0), _zip_streams(k1, v1)))
            else:
                _start(_merge(v0, v1))

        cx = pltpu.make_async_copy(x_hbm, x_buf, sem_a)
        cr = pltpu.make_async_copy(wr_hbm, wr_buf, sem_a)
        wq_c = [pltpu.make_async_copy(wq_hbm.at[pl.ds(r, 8), pl.ds(c, 2048)],
                                      wq_buf.at[pl.ds(r, 8), pl.ds(c, 2048)], sem_a)
                for r in range(0, D, 8) for c in range(0, H * DH, 2048)]
        k0_small = [head_copies(k_hbm, j, k0_buf.at[j], k_small, sem_a) for j in range(LEAD)]
        k0_big = [head_copies(k_hbm, j, k0_buf.at[j], k_big, sem_a) for j in range(LEAD)]
        wo_early = (H - LEAD) * DH
        _issue([(cx, cr)] + _two(wq_c, row_copies(wo_hbm, wo_buf, sem_b, 0, wo_early)))
        _start(_merge(_zip_streams(*k0_small), _zip_streams(*k0_big)))
        _issue(_two(row_copies(wg_hbm, wg_buf, sem_b, 0, F), row_copies(wu_hbm, wu_buf, sem_b, 0, F))
               + _one(row_copies(wd_hbm, wd_buf, sem_b, 0, F)))
        for g in range(NBUF - 2):
            start_group(g, g)

        cx.wait()
        cr.wait()
        wait_all(wq_buf, sem_a)
        wait_all(k0_buf, sem_a)
        x = x_buf[...].reshape(1, D).astype(F32)
        mu = jnp.mean(x, axis=-1, keepdims=True)
        xc = x - mu
        var = jnp.mean(xc * xc, axis=-1, keepdims=True)
        xn = xc / jnp.sqrt(var + EPS)
        xn_b = xn.astype(BF)
        router = jnp.sum(xn_b.astype(F32) * wr_buf[...].reshape(1, D).astype(F32), axis=-1, keepdims=True)

        q_all = jnp.dot(xn_b, wq_buf[...], preferred_element_type=F32)
        for h in range(H):
            q_scr[h] = q_all[:, h * DH:(h + 1) * DH]

        def scores_softmax(h, k_ref, p_slot):
            q = q_scr[h].astype(BF)
            s = jax.lax.dot_general(q, k_ref[...], NT, preferred_element_type=F32) * (DH ** -0.5)
            e = jnp.exp(s - jnp.max(s, axis=-1, keepdims=True))
            p_scr[p_slot] = (e * (1.0 / jnp.sum(e, axis=-1, keepdims=True))).astype(BF)

        def init_body(j, carry):
            scores_softmax(j, k0_buf.at[j], j)
            return carry

        jax.lax.fori_loop(0, LEAD, init_body, 0)
        start_group(NBUF - 2, NBUF - 2)

        wait_all(wg_buf, sem_b)
        wait_all(wu_buf, sem_b)
        wait_all(wd_buf, sem_b)
        wait_all(wo_buf.at[pl.ds(0, wo_early)], sem_b)
        gt = jax.lax.dot_general(xn_b, wg_buf[...], NT, preferred_element_type=F32)
        up = jax.lax.dot_general(xn_b, wu_buf[...], NT, preferred_element_type=F32)
        y = jnp.dot((gt * jax.nn.sigmoid(gt) * up).astype(BF), wd_buf[...], preferred_element_type=F32)
        routed = xn + (xn * 0.0 + y * jax.nn.sigmoid(router))
        gate = routed * jax.nn.sigmoid(routed)

        def p_times_v(slot, p_slot):
            return jnp.dot(p_scr[p_slot], v_buf[slot], preferred_element_type=F32).astype(BF)

        def body(g, acc):
            ng = g + NBUF - 1
            nslot = jax.lax.rem(ng, NBUF)

            @pl.when(ng < H - LEAD)
            def _():
                start_group(ng, nslot)

            @pl.when(ng >= H - LEAD)
            def _():
                start_group(ng, nslot, with_k=False)

            @pl.when(ng == H - 1)
            def _():
                _issue(_pairs(row_copies(wo_hbm, wo_buf, sem_b, wo_early, H * DH), 2))

            slot = jax.lax.rem(g, NBUF)
            wait_all(k_buf.at[slot], sems.at[slot])
            wait_all(v_buf.at[slot], sems.at[slot])
            wo_h = wo_buf[pl.ds(pl.multiple_of(g * DH, DH), DH), :]
            acc = acc + jnp.dot(p_times_v(slot, jax.lax.rem(g, n_p)), wo_h, preferred_element_type=F32)
            scores_softmax(g + LEAD, k_buf.at[slot], jax.lax.rem(g + LEAD, n_p))
            return acc

        acc = jax.lax.fori_loop(0, H - LEAD, body, jnp.zeros((1, D), F32))

        outs = []
        for g in range(H - LEAD, H):
            wait_all(v_buf.at[g % NBUF], sems.at[g % NBUF])
            outs.append(p_times_v(g % NBUF, g % n_p))
        wait_all(wo_buf.at[pl.ds(wo_early, LEAD * DH)], sem_b)
        for g, o in zip(range(H - LEAD, H), outs):
            acc = acc + jnp.dot(o, wo_buf[g * DH:(g + 1) * DH, :], preferred_element_type=F32)
        o_ref[...] = (x + acc * gate).astype(o_ref.dtype).reshape(1, 1, D)

    def fn(A_x, A_k_cache, A_v_cache, A_wq, A_wo, B_x, B_w_r, B_w_gate, B_w_up, B_w_down):
        del B_x
        win = min(4096, max(256, A_k_cache.shape[2] // 4))
        hbm = pl.BlockSpec(memory_space=pltpu.HBM)
        return pl.pallas_call(
            kernel,
            out_shape=jax.ShapeDtypeStruct((1, 1, D), A_x.dtype),
            in_specs=[hbm] * 9,
            out_specs=pl.BlockSpec(memory_space=pltpu.VMEM),
            scratch_shapes=[
                pltpu.VMEM((1, 1, D), BF), pltpu.VMEM((D,), BF),
                pltpu.VMEM((D, H * DH), BF), pltpu.VMEM((H * DH, D), BF),
                pltpu.VMEM((F, D), BF), pltpu.VMEM((F, D), BF), pltpu.VMEM((F, D), BF),
                pltpu.VMEM((LEAD, win, DH), BF), pltpu.VMEM((NBUF, win, DH), BF), pltpu.VMEM((NBUF, win, DH), BF),
                pltpu.VMEM((H, 1, DH), F32), pltpu.VMEM((LEAD + 1, 1, win), BF),
                pltpu.SemaphoreType.DMA((NBUF + 2,)),
            ],
            name=name,
            compiler_params=pltpu.CompilerParams(vmem_limit_bytes=64 * 1024 * 1024, disable_bounds_checks=nobc),
        )(A_x, A_k_cache, A_v_cache, A_wq, A_wo, B_w_r, B_w_gate.T, B_w_up.T, B_w_down)

    return fn


_impl = make(tk=128,tv=64,nobc=False)


@jax.jit
def pallas_recurrent_scan__sliding_block_cached__moe_arch_mod__decode_kernel(
    A_x, A_k_cache, A_v_cache, A_wq, A_wo, B_x, B_w_r, B_w_gate, B_w_up, B_w_down,
):
    return _impl(A_x, A_k_cache, A_v_cache, A_wq, A_wo, B_x, B_w_r, B_w_gate, B_w_up, B_w_down)
```

```python
import jax
import jax.numpy as jnp
from jax.experimental import pallas as pl
from jax.experimental.pallas import tpu as pltpu

H, DH, D, F = 32, 128, 512, 1376
EPS = 1e-5
NT = (((1,), (1,)), ((), ()))
BF, F32 = jnp.bfloat16, jnp.float32

SMALL, BIG = 128, 256
N_BIG, SKIP = 11, 4
K_GRID, V_GRID = 128, 64
WROWS = 32
STRIDE = 8
NBUF = 3
LEAD = 2


def _cut(lo, hi, t, step):
    cuts = sorted({lo, hi, *range(lo + (t - lo) % step, hi, step)})
    return [(a, b - a) for a, b in zip(cuts[:-1], cuts[1:])]


def _split_window(rows, t):
    lo = t % BIG + SKIP * BIG
    hi = lo + N_BIG * BIG
    assert hi <= rows
    return _cut(0, lo, t, SMALL) + _cut(hi, rows, t, SMALL), _cut(lo, hi, t, BIG)


def _zip_lists(*lists):
    return [l[i] for i in range(max(map(len, lists))) for l in lists if i < len(l)]


def _start_merged(q0, q1):
    i = j = 0
    while i < len(q0) or j < len(q1):
        if j >= len(q1) or (i < len(q0) and i * len(q1) <= j * len(q0)):
            q0[i].start(priority=0)
            i += 1
        else:
            q1[j].start(priority=1)
            j += 1


def _pairs(xs, s):
    l0 = [x for c, x in enumerate(xs) if (c // s) % 2 == 0]
    l1 = [x for c, x in enumerate(xs) if (c // s) % 2 == 1]
    m = min(len(l0), len(l1))
    rest = l0[m:] + l1[m:]
    return list(zip(l0, l1)) + [tuple(rest[i:i + 2]) for i in range(0, len(rest), 2)]


def _start_pairs(*pair_lists):
    for pair in _zip_lists(*pair_lists):
        for queue, copy in enumerate(pair):
            copy.start(priority=queue)


def _kernel(x_hbm, k_hbm, v_hbm, wq_hbm, wo_hbm, wr_hbm, wg_hbm, wu_hbm, wd_hbm,
            o_ref,
            x_buf, wr_buf, wq_buf, wo_buf, wg_buf, wu_buf, wd_buf,
            k0_buf, k_buf, v_buf, q_scr, p_scr, sems):
    win = k_buf.shape[1]
    s0 = k_hbm.shape[2] - win
    sem_a, sem_b = sems.at[NBUF], sems.at[NBUF + 1]
    k_small, k_big = _split_window(win, K_GRID)
    v_small, v_big = _split_window(win, V_GRID)
    n_p = LEAD + 1
    wo_early = (H - LEAD) * DH

    def head_copies(hbm, h, dst, pieces, sem):
        return [pltpu.make_async_copy(hbm.at[0, h, pl.ds(s0 + r, n), :], dst.at[pl.ds(r, n)], sem)
                for r, n in pieces]

    def row_copies(src, dst, sem, lo, hi):
        return [pltpu.make_async_copy(src.at[pl.ds(r, WROWS), :], dst.at[pl.ds(r, WROWS), :], sem)
                for r in range(lo, hi, WROWS)]

    def wait_all(buf, sem):
        pltpu.make_async_copy(buf, buf, sem).wait()

    def start_group(g, slot, with_k):
        sem = sems.at[slot]
        v0 = head_copies(v_hbm, g, v_buf.at[slot], v_small, sem)
        v1 = head_copies(v_hbm, g, v_buf.at[slot], v_big, sem)
        if with_k:
            k0 = head_copies(k_hbm, g + LEAD, k_buf.at[slot], k_small, sem)
            k1 = head_copies(k_hbm, g + LEAD, k_buf.at[slot], k_big, sem)
            _start_merged(_zip_lists(k0, v0), _zip_lists(k1, v1))
        else:
            _start_merged(v0, v1)

    cx = pltpu.make_async_copy(x_hbm, x_buf, sem_a)
    cr = pltpu.make_async_copy(wr_hbm, wr_buf, sem_a)
    cx.start(priority=0)
    cr.start(priority=1)
    wq_c = [pltpu.make_async_copy(wq_hbm.at[pl.ds(r, 8), pl.ds(c, 2048)],
                                  wq_buf.at[pl.ds(r, 8), pl.ds(c, 2048)], sem_a)
            for r in range(0, D, 8) for c in range(0, H * DH, 2048)]
    _start_pairs(_pairs(wq_c, STRIDE), _pairs(row_copies(wo_hbm, wo_buf, sem_b, 0, wo_early), STRIDE))
    _start_merged(_zip_lists(*[head_copies(k_hbm, j, k0_buf.at[j], k_small, sem_a) for j in range(LEAD)]),
                  _zip_lists(*[head_copies(k_hbm, j, k0_buf.at[j], k_big, sem_a) for j in range(LEAD)]))
    _start_pairs(_pairs(row_copies(wg_hbm, wg_buf, sem_b, 0, F), STRIDE),
                 _pairs(row_copies(wu_hbm, wu_buf, sem_b, 0, F), STRIDE))
    wd_c = row_copies(wd_hbm, wd_buf, sem_b, 0, F)
    half = (len(wd_c) // 2 + 1) // 2 * 2
    _start_pairs(_pairs(wd_c[:half], STRIDE), _pairs(wd_c[half:], STRIDE))
    for g in range(NBUF - 2):
        start_group(g, g, True)

    cx.wait()
    cr.wait()
    wait_all(wq_buf, sem_a)
    wait_all(k0_buf, sem_a)
    x = x_buf[...].reshape(1, D).astype(F32)
    xc = x - jnp.mean(x, axis=-1, keepdims=True)
    var = jnp.mean(xc * xc, axis=-1, keepdims=True)
    xn = xc / jnp.sqrt(var + EPS)
    xn_b = xn.astype(BF)
    router = jnp.sum(xn_b.astype(F32) * wr_buf[...].reshape(1, D).astype(F32), axis=-1, keepdims=True)

    q_all = jnp.dot(xn_b, wq_buf[...], preferred_element_type=F32)
    for h in range(H):
        q_scr[h] = q_all[:, h * DH:(h + 1) * DH]

    def scores_softmax(h, k_ref, p_slot):
        q = q_scr[h].astype(BF)
        s = jax.lax.dot_general(q, k_ref[...], NT, preferred_element_type=F32) * (DH ** -0.5)
        e = jnp.exp(s - jnp.max(s, axis=-1, keepdims=True))
        p_scr[p_slot] = (e * (1.0 / jnp.sum(e, axis=-1, keepdims=True))).astype(BF)

    def init_body(j, carry):
        scores_softmax(j, k0_buf.at[j], j)
        return carry

    jax.lax.fori_loop(0, LEAD, init_body, 0)
    start_group(NBUF - 2, NBUF - 2, True)

    wait_all(wg_buf, sem_b)
    wait_all(wu_buf, sem_b)
    wait_all(wd_buf, sem_b)
    wait_all(wo_buf.at[pl.ds(0, wo_early)], sem_b)
    gt = jax.lax.dot_general(xn_b, wg_buf[...], NT, preferred_element_type=F32)
    up = jax.lax.dot_general(xn_b, wu_buf[...], NT, preferred_element_type=F32)
    y = jnp.dot((gt * jax.nn.sigmoid(gt) * up).astype(BF), wd_buf[...], preferred_element_type=F32)
    routed = xn + (xn * 0.0 + y * jax.nn.sigmoid(router))
    gate = routed * jax.nn.sigmoid(routed)

    def p_times_v(slot, p_slot):
        return jnp.dot(p_scr[p_slot], v_buf[slot], preferred_element_type=F32).astype(BF)

    def body(g, acc):
        ng = g + NBUF - 1
        nslot = jax.lax.rem(ng, NBUF)

        @pl.when(ng < H - LEAD)
        def _():
            start_group(ng, nslot, True)

        @pl.when(ng >= H - LEAD)
        def _():
            start_group(ng, nslot, False)

        @pl.when(ng == H - 1)
        def _():
            _start_pairs(_pairs(row_copies(wo_hbm, wo_buf, sem_b, wo_early, H * DH), 2))

        slot = jax.lax.rem(g, NBUF)
        wait_all(k_buf.at[slot], sems.at[slot])
        wait_all(v_buf.at[slot], sems.at[slot])
        wo_h = wo_buf[pl.ds(pl.multiple_of(g * DH, DH), DH), :]
        acc = acc + jnp.dot(p_times_v(slot, jax.lax.rem(g, n_p)), wo_h, preferred_element_type=F32)
        scores_softmax(g + LEAD, k_buf.at[slot], jax.lax.rem(g + LEAD, n_p))
        return acc

    acc = jax.lax.fori_loop(0, H - LEAD, body, jnp.zeros((1, D), F32))

    outs = []
    for g in range(H - LEAD, H):
        wait_all(v_buf.at[g % NBUF], sems.at[g % NBUF])
        outs.append(p_times_v(g % NBUF, g % n_p))
    wait_all(wo_buf.at[pl.ds(wo_early, LEAD * DH)], sem_b)
    for g, o in zip(range(H - LEAD, H), outs):
        acc = acc + jnp.dot(o, wo_buf[g * DH:(g + 1) * DH, :], preferred_element_type=F32)
    o_ref[...] = (x + acc * gate).astype(o_ref.dtype).reshape(1, 1, D)


@jax.jit
def pallas_recurrent_scan__sliding_block_cached__moe_arch_mod__decode_kernel(
    A_x, A_k_cache, A_v_cache, A_wq, A_wo, B_x, B_w_r, B_w_gate, B_w_up, B_w_down,
):
    del B_x
    win = min(4096, max(256, A_k_cache.shape[2] // 4))
    hbm = pl.BlockSpec(memory_space=pltpu.HBM)
    return pl.pallas_call(
        _kernel,
        out_shape=jax.ShapeDtypeStruct((1, 1, D), A_x.dtype),
        in_specs=[hbm] * 9,
        out_specs=pl.BlockSpec(memory_space=pltpu.VMEM),
        scratch_shapes=[
            pltpu.VMEM((1, 1, D), BF), pltpu.VMEM((D,), BF),
            pltpu.VMEM((D, H * DH), BF), pltpu.VMEM((H * DH, D), BF),
            pltpu.VMEM((F, D), BF), pltpu.VMEM((F, D), BF), pltpu.VMEM((F, D), BF),
            pltpu.VMEM((LEAD, win, DH), BF),
            pltpu.VMEM((NBUF, win, DH), BF), pltpu.VMEM((NBUF, win, DH), BF),
            pltpu.VMEM((H, 1, DH), F32), pltpu.VMEM((LEAD + 1, 1, win), BF),
            pltpu.SemaphoreType.DMA((NBUF + 2,)),
        ],
        compiler_params=pltpu.CompilerParams(vmem_limit_bytes=64 * 1024 * 1024),
    )(A_x, A_k_cache, A_v_cache, A_wq, A_wo, B_w_r, B_w_gate.T, B_w_up.T, B_w_down)
```
